```python
import os as _os
_os.environ.setdefault("JAX_PLATFORMS", "cpu")
import jax
import jax.numpy as jnp

def _softmax(x, axis=-1):
    return jax.nn.softmax(x, axis=axis)
def _gelu(x):
    return jax.nn.gelu(x, approximate=True)
def _silu(x):
    return jax.nn.silu(x)
def _sigmoid(x):
    return jax.nn.sigmoid(x)
def _layernorm(x, axis=-1, eps=1e-5):
    m = jnp.mean(x, axis=axis, keepdims=True)
    v = jnp.var(x, axis=axis, keepdims=True)
    return (x - m) / jnp.sqrt(v + eps)
def _scatter_add(tgt, idx, src, axis=0):
    return tgt.at[idx].add(src)
def _segment_sum(src, seg, n):
    return jax.ops.segment_sum(src, seg, n)
class _Rng:
    def __init__(self, key):
        self._k = key
    def _next(self):
        self._k, sub = jax.random.split(self._k)
        return sub
    def normal(self, shape):
        return jax.random.normal(self._next(), shape, dtype=jnp.bfloat16)
    def randint(self, lo, hi, shape):
        return jax.random.randint(self._next(), shape, lo, hi, dtype=jnp.int32)
    def uniform(self, shape, lo=0.0, hi=1.0):
        return jax.random.uniform(self._next(), shape, jnp.bfloat16, lo, hi)
    def permutation(self, n):
        return jax.random.permutation(self._next(), n)


kernel_name = 'sequential_preLN__sliding_block_cached__mixer_channel_mlp__decode'

def setup_inputs():
    _rng = _Rng(jax.random.key(int.from_bytes(__import__("os").urandom(4), "little")))
    _w = (lambda a: (lambda t: t.astype(jnp.bfloat16) if jnp.issubdtype(t.dtype, jnp.floating) else t)(jnp.asarray(a)))
    def _A_setup():
        B, Sq, D = 1, 1, 512
        Hq, Hkv, Sk, Dh = 32, 8, 65536, 128
        assert Hq % Hkv == 0, (Hq, Hkv)
        return {
            "x": _w((lambda *s: _rng.normal(s) * 0.05)(B, Sq, D)),
            "k_cache": _w((lambda *s: _rng.normal(s) * 3.2)(B, Hkv, Sk, Dh)),
            "v_cache": _w((lambda *s: _rng.normal(s) * 0.2)(B, Hkv, Sk, Dh)),
            "wq": _w((lambda *s: _rng.normal(s) * 3.2)(D, Hq * Dh) * (D ** -0.5)),
            "wo": _w((lambda *s: _rng.normal(s) * 0.2)(Hq * Dh, D) * ((Hq * Dh) ** -0.5)),
        }
    _A_in = _A_setup()

    def _B_setup():
        B, S, D, F = 1, 1, 512, 1792
        return {
            "x": _w((lambda *s: _rng.normal(s) * 0.05)(B, S, D)),
            "w1": _w((lambda *s: _rng.normal(s) * 0.2)(D, F) * (D ** -0.5)),
            "b1": _w((lambda *s: _rng.normal(s) * 0.2)(F)),
            "w2": _w((lambda *s: _rng.normal(s) * 0.2)(F, D) * (F ** -0.5)),
            "b2": _w((lambda *s: _rng.normal(s) * 0.05)(D)),
        }
    _B_in = _B_setup()

    return {
        "A_x": _A_in["x"],
        "A_k_cache": _A_in["k_cache"],
        "A_v_cache": _A_in["v_cache"],
        "A_wq": _A_in["wq"],
        "A_wo": _A_in["wo"],
        "B_x": _B_in["x"],
        "B_w1": _B_in["w1"],
        "B_b1": _B_in["b1"],
        "B_w2": _B_in["w2"],
        "B_b2": _B_in["b2"],
    }

def reference(A_x, A_k_cache, A_v_cache, A_wq, A_wo, B_x, B_w1, B_b1, B_w2, B_b2):
    def _A_ref(x, k_cache, v_cache, wq, wo):
        B, Sq, D = x.shape
        Hq, Dh = 32, 128
        Hkv, Sk = k_cache.shape[1], k_cache.shape[2]
        W = min(4096, max(256, Sk // 4))
        rep = Hq // Hkv
        q = (lambda x, *d: x.transpose(*d))((x @ wq).reshape(B, Sq, Hq, Dh), 0, 2, 1, 3)
        k = jnp.repeat(k_cache[:, :, Sk - W:, :], rep, axis=1)
        v = jnp.repeat(v_cache[:, :, Sk - W:, :], rep, axis=1)
        scores = jnp.einsum("bhqd,bhkd->bhqk", q, k) * (Dh ** -0.5)
        p = _softmax(scores, axis=-1)
        o = jnp.einsum("bhqk,bhkd->bhqd", p, v)
        return (lambda x, *d: x.transpose(*d))(o, 0, 2, 1, 3).reshape(B, Sq, Hq * Dh) @ wo

    def _B_ref(x, w1, b1, w2, b2):
        y = _layernorm(x, axis=-1)
        h = _gelu(jnp.einsum("bsd,df->bsf", y, w1) + b1)
        return jnp.einsum("bsf,fd->bsd", h, w2) + b2

    x = A_x
    h = x + _A_ref(_layernorm(x, axis=-1), A_k_cache, A_v_cache, A_wq, A_wo)
    h2 = h + _B_ref(_layernorm(h, axis=-1), B_w1, B_b1, B_w2, B_b2)
    return h2
```

```python
import functools
import numpy as np
import jax
import jax.numpy as jnp
from jax import lax
import jax.experimental.pallas as pl
import jax.experimental.pallas.tpu as pltpu

D, HQ, HKV, DH, F = 512, 32, 8, 128, 1792
REP = HQ // HKV
BF, F32 = jnp.bfloat16, jnp.float32
mo = pl.multiple_of


def _ln(t):
    m = jnp.mean(t, axis=-1, keepdims=True)
    c = t - m
    v = jnp.mean(c * c, axis=-1, keepdims=True)
    return c * lax.rsqrt(v + 1e-5)


def make(lead=6, qsplit=2, w2_groups=(4, 4, 3, 2, 1), bias_2d=True, checks=False, M=8):
    def kern(x_hbm, k_hbm, v_hbm, wq_hbm, wo_hbm, w1_hbm, b1_hbm, w2_hbm, b2_hbm, o_ref,
             xb, b1b, b2b, kb, vb, wqb, wob, w1b, w2b, qs, s_small, s_w, s_k, s_v, s_w2):
        SK = k_hbm.shape[2]
        W = min(4096, max(256, SK // 4))
        NR = W // 128

        def issue_a(i):
            for j in range(8):
                idx = j * 16 + i
                r = mo((idx // 2) * 8, 8)
                col = mo((idx % 2) * 2048, 2048)
                pltpu.make_async_copy(wq_hbm.at[pl.ds(r, 8), pl.ds(col, 2048)],
                                      wqb.at[pl.ds(r, 8), pl.ds(col, 2048)], s_w.at[0]).start(priority=0)
                r = mo(idx * 32, 32)
                pltpu.make_async_copy(wo_hbm.at[pl.ds(r, 32)], wob.at[pl.ds(r, 32)], s_w.at[1]).start(priority=1)

        def issue_b(i):
            r = mo(SK - W + i * 128, 128)
            for h in range(HKV):
                pltpu.make_async_copy(k_hbm.at[0, h, pl.ds(r, 128)], kb.at[i, h], s_k.at[i]).start(priority=0)
                pltpu.make_async_copy(v_hbm.at[0, h, pl.ds(r, 128)], vb.at[i, h], s_v.at[i]).start(priority=1)

        def issue_c(i):
            for u in range(2):
                for j in range(8):
                    r = mo((j * 8 + i * 2 + u) * 8, 8)
                    pltpu.make_async_copy(w1_hbm.at[pl.ds(r, 8)], w1b.at[pl.ds(r, 8)], s_w.at[2]).start(priority=j % 2)

        starts = np.cumsum((0,) + tuple(w2_groups))

        def issue_d(g):
            n = w2_groups[g]
            t = 0
            for p in range(4):
                for m in range(n):
                    r = (int(starts[g]) + m) * 128 + p * 32
                    pltpu.make_async_copy(w2_hbm.at[pl.ds(r, 32)], w2b.at[pl.ds(r, 32)], s_w2.at[g]).start(priority=t % 2)
                    t += 1

        small = [pltpu.make_async_copy(x_hbm, xb, s_small.at[0]),
                 pltpu.make_async_copy(b1_hbm, b1b, s_small.at[1]),
                 pltpu.make_async_copy(b2_hbm, b2b, s_small.at[2])]

        issue_a(0)
        for c in small:
            c.start()
        pl.loop(1, 16)(issue_a)
        pl.loop(0, lead)(issue_b)

        for c in small:
            c.wait()
        x = xb[0].astype(F32)
        y = jnp.broadcast_to(_ln(x), (M, D)).astype(BF)
        pltpu.make_async_copy(wqb, wqb, s_w.at[0]).wait()

        row = lax.broadcasted_iota(jnp.int32, (M, DH), 0) % REP
        gper = HKV // qsplit

        @pl.loop(0, qsplit)
        def _(t):
            issue_b(lead + t)
            for gg in range(gper):
                g = t * gper + gg
                q = jnp.dot(y, wqb[:, pl.ds(mo(g * REP * DH, REP * DH), REP * DH)], preferred_element_type=F32)
                qg = q[:, 0:DH]
                for r in range(1, REP):
                    qg = jnp.where(row == r, q[:, r * DH:(r + 1) * DH], qg)
                qs[g] = qg

        first = lead + qsplit
        scale = DH ** -0.5
        qv = [qs[g].astype(BF) for g in range(HKV)]

        def att(c, carry):
            nxt = c + first

            @pl.when(nxt < NR)
            def _():
                issue_b(nxt)

            @pl.when(jnp.logical_and(nxt >= NR, nxt < NR + 4))
            def _():
                issue_c(nxt - NR)

            ng = len(w2_groups)
            slots = first - 4
            for sl in range(slots):
                gs = [g for g in range(ng) if min(g, slots - 1) == sl]

                @pl.when(nxt == NR + 4 + sl)
                def _():
                    for g in gs:
                        issue_d(g)

            pltpu.make_async_copy(kb.at[c], kb.at[c], s_k.at[c]).wait()
            pltpu.make_async_copy(vb.at[c], vb.at[c], s_v.at[c]).wait()
            ss = [lax.dot_general(qv[h], kb[c, h], (((1,), (1,)), ((), ())), preferred_element_type=F32) * scale
                  for h in range(HKV)]
            st = []
            for h in range(HKV):
                m, l, acc = carry[h]
                mn = jnp.maximum(m, jnp.max(ss[h], axis=-1, keepdims=True))
                a = jnp.exp(m - mn)
                p = jnp.exp(ss[h] - mn)
                st.append((mn, a, p))
            out = []
            for h in range(HKV):
                m, l, acc = carry[h]
                mn, a, p = st[h]
                out.append((mn, a * l + p, a * acc + jnp.dot(p.astype(BF), vb[c, h], preferred_element_type=F32)))
            return tuple(out)

        init = tuple((jnp.full((M, DH), -jnp.inf, F32), jnp.zeros((M, DH), F32), jnp.zeros((M, DH), F32))
                     for _ in range(HKV))
        fin = lax.fori_loop(0, NR, att, init)

        pltpu.make_async_copy(wob, wob, s_w.at[1]).wait()
        attn = jnp.zeros((M, D), F32)
        for h in range(HKV):
            m, l, acc = fin[h]
            o = acc / jnp.sum(l, axis=-1, keepdims=True)
            lhs = jnp.concatenate([jnp.broadcast_to(o[r:r + 1], (M, DH)) for r in range(REP)], axis=1).astype(BF)
            attn = attn + jnp.dot(lhs, wob[pl.ds(h * REP * DH, REP * DH), :], preferred_element_type=F32)
        hres = x + attn
        y2 = _ln(_ln(hres)).astype(BF)

        pltpu.make_async_copy(w1b, w1b, s_w.at[2]).wait()
        u = jnp.dot(y2, w1b[...], preferred_element_type=F32)
        if bias_2d:
            b1 = b1b[...].astype(F32)
            b1 = jnp.concatenate([b1[j:j + 1] for j in range(F // 128)], axis=1)
            b2 = b2b[...].astype(F32)
            b2 = jnp.concatenate([b2[j:j + 1] for j in range(D // 128)], axis=1)
        else:
            b1 = b1b[...].astype(F32).reshape(1, F)
            b2 = b2b[...].astype(F32).reshape(1, D)
        gl = jax.nn.gelu(u + b1, approximate=True).astype(BF)
        res = hres + b2
        for g, n in enumerate(w2_groups):
            r0 = int(starts[g]) * 128
            blk = w2b.at[pl.ds(r0, n * 128)]
            pltpu.make_async_copy(blk, blk, s_w2.at[g]).wait()
            res = res + jnp.dot(gl[:, r0:r0 + n * 128], blk[...], preferred_element_type=F32)
        o_ref[0] = res[0:1].astype(o_ref.dtype)

    def fn(A_x, A_k_cache, A_v_cache, A_wq, A_wo, B_x, B_w1, B_b1, B_w2, B_b2):
        hbm = pl.BlockSpec(memory_space=pltpu.HBM)
        b1s, b2s = ((F // 128, 128), (D // 128, 128)) if bias_2d else ((F,), (D,))
        dma = pltpu.SemaphoreType.DMA
        return pl.pallas_call(
            kern,
            in_specs=[hbm] * 9,
            out_specs=pl.BlockSpec(memory_space=pltpu.VMEM),
            out_shape=jax.ShapeDtypeStruct((1, 1, D), A_x.dtype),
            scratch_shapes=[
                pltpu.VMEM((1, 1, D), BF), pltpu.VMEM(b1s, BF), pltpu.VMEM(b2s, BF),
                pltpu.VMEM((32, HKV, 128, DH), BF), pltpu.VMEM((32, HKV, 128, DH), BF),
                pltpu.VMEM((D, HQ * DH), BF), pltpu.VMEM((HQ * DH, D), BF),
                pltpu.VMEM((D, F), BF), pltpu.VMEM((F, D), BF),
                pltpu.VMEM((HKV, M, DH), F32),
                dma((3,)), dma((3,)), dma((32,)), dma((32,)), dma((len(w2_groups),)),
            ],
            compiler_params=pltpu.CompilerParams(
                vmem_limit_bytes=64 * 2**20,
                disable_semaphore_checks=not checks, disable_bounds_checks=not checks),
        )(A_x, A_k_cache, A_v_cache, A_wq, A_wo, B_w1, B_b1.reshape(b1s), B_w2, B_b2.reshape(b2s))
    return fn


@jax.jit
def pallas_sequential_preLN__sliding_block_cached__mixer_channel_mlp__decode_kernel(
        A_x, A_k_cache, A_v_cache, A_wq, A_wo, B_x, B_w1, B_b1, B_w2, B_b2):
    return make(lead=5, qsplit=1)(A_x, A_k_cache, A_v_cache, A_wq, A_wo, B_x, B_w1, B_b1, B_w2, B_b2)
```

```python
import functools

import jax
import jax.numpy as jnp
import numpy as np
from jax import lax
import jax.experimental.pallas as pl
import jax.experimental.pallas.tpu as pltpu

D, HQ, HKV, DH, F = 512, 32, 8, 128, 1792
REP = HQ // HKV
WINDOW = 4096
EPS = 1e-5
ROWS = 8

KEYS = 128
N_KV = WINDOW // KEYS
N_W = 16
N_MLP = 56
W2_ROWS = F // N_MLP

HEAD_WQ, HEAD_K = 3, 1
HEAD_P0 = 2
LEAD = 3
Q_STEPS = 2
WO_PARTS = 4
WO_ISSUE = (1, 1, 0, 1)
BATCH = 16

W1_ORDER = tuple((28 + 19 * i) % N_MLP for i in range(N_MLP))
W2_ORDER = tuple((19 * i) % N_MLP for i in range(N_MLP))
W2_ON_P0 = 18
W2_SMALL = 7
W2_MXU = (32, 12)
W2_VPU = (4, 4, 3, 1)
W2_BOUNDS = tuple(int(b) for b in np.cumsum((0,) + W2_MXU + W2_VPU))

SEM_X, SEM_B1, SEM_B2, SEM_WQ, SEM_W1, SEM_WO = range(6)
SEM_K = SEM_WO + WO_PARTS
SEM_V = SEM_K + N_KV
SEM_W2 = SEM_V + N_KV
N_SEMS = SEM_W2 + len(W2_BOUNDS) - 1


def _aligned(i, m):
    return i if isinstance(i, int) else pl.multiple_of(i, m)


def _layernorm(t):
    c = t - jnp.mean(t, axis=-1, keepdims=True)
    return c * lax.rsqrt(jnp.mean(c * c, axis=-1, keepdims=True) + EPS)


def _alternate(p0, p1):
    out = []
    for t in range(max(len(p0), len(p1))):
        out += [(q[t], prio) for prio, q in enumerate((p0, p1)) if t < len(q)]
    return out


def _block_kernel(x_hbm, k_hbm, v_hbm, wq_hbm, wo_hbm, w1_hbm, b1_hbm, w2_hbm, b2_hbm, o_ref,
                  x_buf, b1_buf, b2_buf, k_buf, v_buf, wq_buf, wo_buf, w1_buf, w2_buf, q_buf, sems):
    f32, bf16 = jnp.float32, jnp.bfloat16
    first_key = k_hbm.shape[2] - WINDOW

    def start(src, dst, sem, prio):
        pltpu.make_async_copy(src, dst, sems.at[sem]).start(priority=prio)

    def wait_filled(buf, sem):
        pltpu.make_async_copy(buf, buf, sems.at[sem]).wait()

    def wq_chunk(i, j, prio):
        half = HQ * DH // 2
        at = (pl.ds(_aligned(j * (D // 8) + (i // 2) * 8, 8), 8), pl.ds(_aligned((i % 2) * half, half), half))
        start(wq_hbm.at[at], wq_buf.at[at], SEM_WQ, prio)

    def wo_chunk(i, j, prio):
        per_part = N_W // WO_PARTS
        src = wo_hbm.at[pl.ds(_aligned(j * REP * DH + i * 32, 32), 32)]
        dst = wo_buf.at[i // per_part, j, pl.ds(_aligned((i % per_part) * 32, 32), 32)]
        start(src, dst, SEM_WO + i // per_part, prio)

    def k_chunk(i, h, prio):
        start(k_hbm.at[0, h, pl.ds(_aligned(first_key + i * KEYS, KEYS), KEYS)], k_buf.at[i, h], SEM_K + i, prio)

    def v_chunk(i, h, prio):
        start(v_hbm.at[0, h, pl.ds(_aligned(first_key + i * KEYS, KEYS), KEYS)], v_buf.at[i, h], SEM_V + i, prio)

    def w1_chunk(c, prio):
        per_row = F // 128
        r, t = divmod(16 * c, per_row)
        for row, lo, n in ((r, t, per_row - t), (r + 1, 0, 16 - per_row + t)):
            at = (pl.ds(row * 8, 8), pl.ds(lo * 128, n * 128))
            start(w1_hbm.at[at], w1_buf.at[at], SEM_W1, prio)

    def w2_chunk(i, lo, n, prio):
        c = W2_ORDER[i]
        slot = (i // 4) * 4 + c % 4 if i < sum(W2_MXU) else i
        group = sum(b <= i for b in W2_BOUNDS[1:])
        start(w2_hbm.at[pl.ds(c * W2_ROWS + lo, n)], w2_buf.at[pl.ds(slot * W2_ROWS + lo, n)], SEM_W2 + group, prio)

    def issue_round(chunk0, i0, chunk1, i1):
        for j in range(8):
            chunk0(i0, j, 0)
            chunk1(i1, j, 1)

    def issue(batch):
        for chunk, prio in batch:
            chunk(prio)

    k_ahead = N_W - HEAD_WQ + HEAD_K
    wo_from = N_KV - k_ahead
    part = functools.partial
    n_whole = N_MLP - W2_SMALL
    on_p0 = range(n_whole - 2 * W2_ON_P0 + 1, n_whole, 2)
    tail = _alternate(
        [part(w1_chunk, c) for c in W1_ORDER] + [part(w2_chunk, i, 0, W2_ROWS) for i in on_p0],
        [part(wo_chunk, i, j) for i in range(N_KV - wo_from, N_W) for j in range(8)]
        + [part(w2_chunk, i, 0, W2_ROWS) for i in range(n_whole) if i not in on_p0]
        + [part(w2_chunk, i, lo, 8) for i in range(n_whole, N_MLP) for lo in range(0, W2_ROWS, 8)])
    batches = [tail[t:t + BATCH] for t in range(0, len(tail), BATCH)]

    head_wq = [part(wq_chunk, i, j) for i in range(HEAD_WQ) for j in range(8)]
    head_p1 = head_wq[:-HEAD_P0] + [part(k_chunk, i, h) for i in range(HEAD_K) for h in range(HKV)]
    issue([(chunk, 1) for chunk in head_p1[:4]])
    start(x_hbm, x_buf, SEM_X, 0)
    start(b1_hbm, b1_buf, SEM_B1, 0)
    start(b2_hbm, b2_buf, SEM_B2, 0)
    issue([(chunk, 1) for chunk in head_p1[4:-HEAD_P0]])
    issue(_alternate(head_wq[-HEAD_P0:], head_p1[-HEAD_P0:]))
    pl.loop(HEAD_WQ, N_W)(lambda i: issue_round(wq_chunk, i, k_chunk, i - HEAD_WQ + HEAD_K))

    wait_filled(x_buf, SEM_X)
    wait_filled(b1_buf, SEM_B1)
    wait_filled(b2_buf, SEM_B2)
    x = x_buf[0].astype(f32)
    y = jnp.broadcast_to(_layernorm(x), (ROWS, D)).astype(bf16)
    pl.loop(0, LEAD)(lambda i: issue_round(v_chunk, i, k_chunk, i + k_ahead))

    wait_filled(wq_buf, SEM_WQ)
    head_of_row = lax.broadcasted_iota(jnp.int32, (ROWS, DH), 0) % REP

    @pl.loop(0, Q_STEPS)
    def _(t):
        issue_round(v_chunk, LEAD + t, k_chunk, LEAD + t + k_ahead)
        for u in range(HKV // Q_STEPS):
            g = t * (HKV // Q_STEPS) + u
            cols = pl.ds(_aligned(g * REP * DH, REP * DH), REP * DH)
            q = jnp.dot(y, wq_buf[:, cols], preferred_element_type=f32)
            rows = q[:, :DH]
            for r in range(1, REP):
                rows = jnp.where(head_of_row == r, q[:, r * DH:(r + 1) * DH], rows)
            q_buf[g] = rows

    ahead = LEAD + Q_STEPS
    qs = [q_buf[g].astype(bf16) for g in range(HKV)]

    def attend(c, carry):
        nxt = c + ahead

        @pl.when(nxt < wo_from)
        def _():
            issue_round(v_chunk, nxt, k_chunk, nxt + k_ahead)

        @pl.when(jnp.logical_and(nxt >= wo_from, nxt < N_KV))
        def _():
            issue_round(v_chunk, nxt, wo_chunk, nxt - wo_from)

        @pl.when(nxt >= N_KV)
        def _():
            for t in range(ahead):
                pl.when(nxt == N_KV + t)(part(issue, batches[t]))

        wait_filled(k_buf.at[c], SEM_K + c)
        wait_filled(v_buf.at[c], SEM_V + c)
        scores = [lax.dot_general(qs[g], k_buf[c, g], (((1,), (1,)), ((), ())), preferred_element_type=f32)
                  * DH ** -0.5 for g in range(HKV)]
        stats = []
        for s, (m, _, _) in zip(scores, carry):
            m_new = jnp.maximum(m, jnp.max(s, axis=-1, keepdims=True))
            stats.append((m_new, jnp.exp(m - m_new), jnp.exp(s - m_new)))
        return tuple(
            (m_new, alpha * l + p,
             alpha * acc + jnp.dot(p.astype(bf16), v_buf[c, g], preferred_element_type=f32))
            for g, ((m_new, alpha, p), (_, l, acc)) in enumerate(zip(stats, carry)))

    zeros = jnp.zeros((ROWS, DH), f32)
    lowest = jnp.full((ROWS, DH), np.finfo(np.float32).min, f32)
    state = lax.fori_loop(0, N_KV, attend, ((lowest, zeros, zeros),) * HKV)

    heads = []
    for _, l, acc in state:
        o = acc / jnp.sum(l, axis=-1, keepdims=True)
        heads += [jnp.broadcast_to(o[r:r + 1], (ROWS, DH)).astype(bf16) for r in range(REP)]
    issued = ahead
    h = jnp.broadcast_to(x, (ROWS, D))
    per_part = REP // WO_PARTS
    for p in range(WO_PARTS):
        for batch in batches[issued:issued + WO_ISSUE[p]]:
            issue(batch)
        issued += WO_ISSUE[p]
        wait_filled(wo_buf.at[p], SEM_WO + p)
        for g in range(HKV):
            lhs = jnp.concatenate(heads[g * REP + p * per_part:g * REP + (p + 1) * per_part], axis=1)
            h = h + jnp.dot(lhs, wo_buf[p, g], preferred_element_type=f32)
    for batch in batches[issued:]:
        issue(batch)

    y2 = _layernorm(_layernorm(h)).astype(bf16)
    b1 = b1_buf[...].astype(f32).reshape(1, F)
    b2 = b2_buf[...].astype(f32).reshape(1, D)
    wait_filled(w1_buf, SEM_W1)
    act = jax.nn.gelu(jnp.dot(y2, w1_buf[...], preferred_element_type=f32) + b1, approximate=True)

    quarter = lax.broadcasted_iota(jnp.int32, (ROWS, 128), 1) // W2_ROWS
    act_tiles = []
    for t in range(0, N_MLP, 4):
        blocks = [act[:, (c // 4) * 128:(c // 4 + 1) * 128] for c in W2_ORDER[t:t + 4]]
        tile = blocks[0]
        for c, block in zip(W2_ORDER[t + 1:t + 4], blocks[1:]):
            tile = jnp.where(quarter == c % 4, block, tile)
        act_tiles.append(tile.astype(bf16))
    act_cols = {}
    for t in range(sum(W2_MXU), N_MLP, 4):
        down = jnp.broadcast_to(act_tiles[t // 4].astype(f32)[:1], (128, 128)).T
        for i in range(t, t + 4):
            lo = (W2_ORDER[i] % 4) * W2_ROWS
            act_cols[i] = down[lo:lo + W2_ROWS]

    out = h + b2
    for group, (lo, hi) in enumerate(zip(W2_BOUNDS, W2_BOUNDS[1:])):
        rows = w2_buf.at[pl.ds(lo * W2_ROWS, (hi - lo) * W2_ROWS)]
        if group == len(W2_MXU):
            out = jnp.where(lax.broadcasted_iota(jnp.int32, (ROWS, D), 0) == 0, out, 0.0)
        wait_filled(rows, SEM_W2 + group)
        if group < len(W2_MXU):
            lhs = jnp.concatenate(act_tiles[lo // 4:hi // 4], axis=1)
            out = out + jnp.dot(lhs, rows[...], preferred_element_type=f32)
            continue
        for i in range(lo, hi):
            w = w2_buf[pl.ds(i * W2_ROWS, W2_ROWS), :].astype(f32)
            t0, t1, t2, t3 = (w[r:r + 8] * jnp.tile(act_cols[i][r:r + 8], (1, D // 128))
                              for r in range(0, W2_ROWS, 8))
            out = out + ((t0 + t1) + (t2 + t3))
    o_ref[0] = jnp.sum(out, axis=0, keepdims=True).astype(o_ref.dtype)


@jax.jit
def pallas_sequential_preLN__sliding_block_cached__mixer_channel_mlp__decode_kernel(
    A_x: jax.Array,
    A_k_cache: jax.Array,
    A_v_cache: jax.Array,
    A_wq: jax.Array,
    A_wo: jax.Array,
    B_x: jax.Array,
    B_w1: jax.Array,
    B_b1: jax.Array,
    B_w2: jax.Array,
    B_b2: jax.Array,
):
    del B_x
    cache_len = A_k_cache.shape[2]
    assert A_x.shape == (1, 1, D) and A_wq.shape == (D, HQ * DH) and B_w1.shape == (D, F)
    assert A_k_cache.shape == A_v_cache.shape == (1, HKV, cache_len, DH)
    assert min(4096, max(256, cache_len // 4)) == WINDOW and cache_len % KEYS == 0

    return pl.pallas_call(
        _block_kernel,
        in_specs=[pl.BlockSpec(memory_space=pltpu.HBM)] * 9,
        out_specs=pl.BlockSpec(memory_space=pltpu.VMEM),
        out_shape=jax.ShapeDtypeStruct(A_x.shape, A_x.dtype),
        scratch_shapes=[
            pltpu.VMEM(A_x.shape, A_x.dtype),
            pltpu.VMEM(B_b1.shape, B_b1.dtype),
            pltpu.VMEM(B_b2.shape, B_b2.dtype),
            pltpu.VMEM((N_KV, HKV, KEYS, DH), A_k_cache.dtype),
            pltpu.VMEM((N_KV, HKV, KEYS, DH), A_v_cache.dtype),
            pltpu.VMEM(A_wq.shape, A_wq.dtype),
            pltpu.VMEM((WO_PARTS, HKV, REP * DH // WO_PARTS, D), A_wo.dtype),
            pltpu.VMEM(B_w1.shape, B_w1.dtype),
            pltpu.VMEM(B_w2.shape, B_w2.dtype),
            pltpu.VMEM((HKV, ROWS, DH), jnp.float32),
            pltpu.SemaphoreType.DMA((N_SEMS,)),
        ],
        compiler_params=pltpu.CompilerParams(
            vmem_limit_bytes=48 * 1024 * 1024,
            disable_semaphore_checks=True,
        ),
    )(A_x, A_k_cache, A_v_cache, A_wq, A_wo, B_w1, B_b1, B_w2, B_b2)
```

```python
import functools

import jax
import jax.numpy as jnp
import numpy as np
from jax import lax
import jax.experimental.pallas as pl
import jax.experimental.pallas.tpu as pltpu

D, HQ, HKV, DH, F = 512, 32, 8, 128, 1792
REP = HQ // HKV
WINDOW = 4096
EPS = 1e-5
ROWS = 8

KEYS = 128
N_KV = WINDOW // KEYS
N_W = 16
N_MLP = 56
W2_ROWS = F // N_MLP

HEAD_WQ, HEAD_K = 3, 1
HEAD_P0 = 2
LEAD = 3
Q_STEPS = 2
WO_PARTS = 4
WO_ISSUE = (1, 1, 0, 1)
BATCH = 16

W1_ORDER = tuple((28 + 19 * i) % N_MLP for i in range(N_MLP))
W2_ORDER = tuple((19 * i) % N_MLP for i in range(N_MLP))
W2_ON_P0 = 18
W2_SMALL = 7
W2_MXU = (32, 12)
W2_VPU = (4, 3, 2, 1, 1, 1)
W2_BOUNDS = tuple(int(b) for b in np.cumsum((0,) + W2_MXU + W2_VPU))

SEM_X, SEM_B1, SEM_B2, SEM_WQ, SEM_W1, SEM_WO = range(6)
SEM_K = SEM_WO + WO_PARTS
SEM_V = SEM_K + N_KV
SEM_W2 = SEM_V + N_KV
N_SEMS = SEM_W2 + len(W2_BOUNDS) - 1


def _aligned(i, m):
    return i if isinstance(i, int) else pl.multiple_of(i, m)


def _layernorm(t):
    c = t - jnp.mean(t, axis=-1, keepdims=True)
    return c * lax.rsqrt(jnp.mean(c * c, axis=-1, keepdims=True) + EPS)


def _alternate(p0, p1):
    out = []
    for t in range(max(len(p0), len(p1))):
        out += [(q[t], prio) for prio, q in enumerate((p0, p1)) if t < len(q)]
    return out


def _block_kernel(x_hbm, k_hbm, v_hbm, wq_hbm, wo_hbm, w1_hbm, b1_hbm, w2_hbm, b2_hbm, o_ref,
                  x_buf, b1_buf, b2_buf, k_buf, v_buf, wq_buf, wo_buf, w1_buf, w2_buf, q_buf, sems):
    f32, bf16 = jnp.float32, jnp.bfloat16
    first_key = k_hbm.shape[2] - WINDOW

    def start(src, dst, sem, prio):
        pltpu.make_async_copy(src, dst, sems.at[sem]).start(priority=prio)

    def wait_filled(buf, sem):
        pltpu.make_async_copy(buf, buf, sems.at[sem]).wait()

    def wq_chunk(i, j, prio):
        half = HQ * DH // 2
        at = (pl.ds(_aligned(j * (D // 8) + (i // 2) * 8, 8), 8), pl.ds(_aligned((i % 2) * half, half), half))
        start(wq_hbm.at[at], wq_buf.at[at], SEM_WQ, prio)

    def wo_chunk(i, j, prio):
        per_part = N_W // WO_PARTS
        src = wo_hbm.at[pl.ds(_aligned(j * REP * DH + i * 32, 32), 32)]
        dst = wo_buf.at[i // per_part, j, pl.ds(_aligned((i % per_part) * 32, 32), 32)]
        start(src, dst, SEM_WO + i // per_part, prio)

    def k_chunk(i, h, prio):
        start(k_hbm.at[0, h, pl.ds(_aligned(first_key + i * KEYS, KEYS), KEYS)], k_buf.at[i, h], SEM_K + i, prio)

    def v_chunk(i, h, prio):
        start(v_hbm.at[0, h, pl.ds(_aligned(first_key + i * KEYS, KEYS), KEYS)], v_buf.at[i, h], SEM_V + i, prio)

    def w1_chunk(c, prio):
        per_row = F // 128
        r, t = divmod(16 * c, per_row)
        for row, lo, n in ((r, t, per_row - t), (r + 1, 0, 16 - per_row + t)):
            at = (pl.ds(row * 8, 8), pl.ds(lo * 128, n * 128))
            start(w1_hbm.at[at], w1_buf.at[at], SEM_W1, prio)

    def w2_chunk(i, lo, n, prio):
        c = W2_ORDER[i]
        slot = (i // 4) * 4 + c % 4 if i < sum(W2_MXU) else i
        group = sum(b <= i for b in W2_BOUNDS[1:])
        start(w2_hbm.at[pl.ds(c * W2_ROWS + lo, n)], w2_buf.at[pl.ds(slot * W2_ROWS + lo, n)], SEM_W2 + group, prio)

    def issue_round(chunk0, i0, chunk1, i1):
        for j in range(8):
            chunk0(i0, j, 0)
            chunk1(i1, j, 1)

    def issue(batch):
        for chunk, prio in batch:
            chunk(prio)

    k_ahead = N_W - HEAD_WQ + HEAD_K
    wo_from = N_KV - k_ahead
    part = functools.partial
    n_whole = N_MLP - W2_SMALL
    on_p0 = range(n_whole - 2 * W2_ON_P0 + 1, n_whole, 2)
    tail = _alternate(
        [part(w1_chunk, c) for c in W1_ORDER] + [part(w2_chunk, i, 0, W2_ROWS) for i in on_p0],
        [part(wo_chunk, i, j) for i in range(N_KV - wo_from, N_W) for j in range(8)]
        + [part(w2_chunk, i, 0, W2_ROWS) for i in range(n_whole) if i not in on_p0]
        + [part(w2_chunk, i, lo, 8) for i in range(n_whole, N_MLP) for lo in range(0, W2_ROWS, 8)])
    batches = [tail[t:t + BATCH] for t in range(0, len(tail), BATCH)]

    head_wq = [part(wq_chunk, i, j) for i in range(HEAD_WQ) for j in range(8)]
    head_p1 = head_wq[:-HEAD_P0] + [part(k_chunk, i, h) for i in range(HEAD_K) for h in range(HKV)]
    issue([(chunk, 1) for chunk in head_p1[:4]])
    vectors = [pltpu.make_async_copy(src, dst, sems.at[sem]) for src, dst, sem in
               ((x_hbm, x_buf, SEM_X), (b1_hbm, b1_buf, SEM_B1), (b2_hbm, b2_buf, SEM_B2))]
    for copy in vectors:
        copy.start()
    issue([(chunk, 1) for chunk in head_p1[4:-HEAD_P0]])
    issue(_alternate(head_wq[-HEAD_P0:], head_p1[-HEAD_P0:]))
    pl.loop(HEAD_WQ, N_W)(lambda i: issue_round(wq_chunk, i, k_chunk, i - HEAD_WQ + HEAD_K))

    for copy in vectors:
        copy.wait()
    x = x_buf[0].astype(f32)
    y = jnp.broadcast_to(_layernorm(x), (ROWS, D)).astype(bf16)
    pl.loop(0, LEAD)(lambda i: issue_round(v_chunk, i, k_chunk, i + k_ahead))

    wait_filled(wq_buf, SEM_WQ)
    head_of_row = lax.broadcasted_iota(jnp.int32, (ROWS, DH), 0) % REP

    @pl.loop(0, Q_STEPS)
    def _(t):
        issue_round(v_chunk, LEAD + t, k_chunk, LEAD + t + k_ahead)
        for u in range(HKV // Q_STEPS):
            g = t * (HKV // Q_STEPS) + u
            cols = pl.ds(_aligned(g * REP * DH, REP * DH), REP * DH)
            q = jnp.dot(y, wq_buf[:, cols], preferred_element_type=f32)
            rows = q[:, :DH]
            for r in range(1, REP):
                rows = jnp.where(head_of_row == r, q[:, r * DH:(r + 1) * DH], rows)
            q_buf[g] = rows

    ahead = LEAD + Q_STEPS
    qs = [q_buf[g].astype(bf16) for g in range(HKV)]

    def attend(c, carry):
        nxt = c + ahead

        @pl.when(nxt < wo_from)
        def _():
            issue_round(v_chunk, nxt, k_chunk, nxt + k_ahead)

        @pl.when(jnp.logical_and(nxt >= wo_from, nxt < N_KV))
        def _():
            issue_round(v_chunk, nxt, wo_chunk, nxt - wo_from)

        @pl.when(nxt >= N_KV)
        def _():
            for t in range(ahead):
                pl.when(nxt == N_KV + t)(part(issue, batches[t]))

        wait_filled(k_buf.at[c], SEM_K + c)
        wait_filled(v_buf.at[c], SEM_V + c)
        scores = [lax.dot_general(qs[g], k_buf[c, g], (((1,), (1,)), ((), ())), preferred_element_type=f32)
                  * DH ** -0.5 for g in range(HKV)]
        stats = []
        for s, (m, _, _) in zip(scores, carry):
            m_new = jnp.maximum(m, jnp.max(s, axis=-1, keepdims=True))
            stats.append((m_new, jnp.exp(m - m_new), jnp.exp(s - m_new)))
        return tuple(
            (m_new, alpha * l + p,
             alpha * acc + jnp.dot(p.astype(bf16), v_buf[c, g], preferred_element_type=f32))
            for g, ((m_new, alpha, p), (_, l, acc)) in enumerate(zip(stats, carry)))

    zeros = jnp.zeros((ROWS, DH), f32)
    lowest = jnp.full((ROWS, DH), np.finfo(np.float32).min, f32)
    state = lax.fori_loop(0, N_KV, attend, ((lowest, zeros, zeros),) * HKV)

    heads = []
    for _, l, acc in state:
        o = acc / jnp.sum(l, axis=-1, keepdims=True)
        heads += [jnp.broadcast_to(o[r:r + 1], (ROWS, DH)).astype(bf16) for r in range(REP)]
    issued = ahead
    h = jnp.broadcast_to(x, (ROWS, D))
    per_part = REP // WO_PARTS
    for p in range(WO_PARTS):
        for batch in batches[issued:issued + WO_ISSUE[p]]:
            issue(batch)
        issued += WO_ISSUE[p]
        wait_filled(wo_buf.at[p], SEM_WO + p)
        for g in range(HKV):
            lhs = jnp.concatenate(heads[g * REP + p * per_part:g * REP + (p + 1) * per_part], axis=1)
            h = h + jnp.dot(lhs, wo_buf[p, g], preferred_element_type=f32)
    for batch in batches[issued:]:
        issue(batch)

    y2 = _layernorm(_layernorm(h)).astype(bf16)
    b1 = b1_buf[...].astype(f32).reshape(1, F)
    b2 = b2_buf[...].astype(f32).reshape(1, D)
    wait_filled(w1_buf, SEM_W1)
    act = jax.nn.gelu(jnp.dot(y2, w1_buf[...], preferred_element_type=f32) + b1, approximate=True)

    quarter = lax.broadcasted_iota(jnp.int32, (ROWS, 128), 1) // W2_ROWS
    act_tiles = []
    for t in range(0, N_MLP, 4):
        blocks = [act[:, (c // 4) * 128:(c // 4 + 1) * 128] for c in W2_ORDER[t:t + 4]]
        tile = blocks[0]
        for c, block in zip(W2_ORDER[t + 1:t + 4], blocks[1:]):
            tile = jnp.where(quarter == c % 4, block, tile)
        act_tiles.append(tile.astype(bf16))
    act_cols = {}
    for t in range(sum(W2_MXU), N_MLP, 4):
        down = jnp.broadcast_to(act_tiles[t // 4].astype(f32)[:1], (128, 128)).T
        for i in range(t, t + 4):
            lo = (W2_ORDER[i] % 4) * W2_ROWS
            act_cols[i] = down[lo:lo + W2_ROWS]

    out = h + b2
    for group, (lo, hi) in enumerate(zip(W2_BOUNDS, W2_BOUNDS[1:])):
        rows = w2_buf.at[pl.ds(lo * W2_ROWS, (hi - lo) * W2_ROWS)]
        if group == len(W2_MXU):
            out = jnp.where(lax.broadcasted_iota(jnp.int32, (ROWS, D), 0) == 0, out, 0.0)
        wait_filled(rows, SEM_W2 + group)
        if group < len(W2_MXU):
            lhs = jnp.concatenate(act_tiles[lo // 4:hi // 4], axis=1)
            out = out + jnp.dot(lhs, rows[...], preferred_element_type=f32)
            continue
        for i in range(lo, hi):
            w = w2_buf[pl.ds(i * W2_ROWS, W2_ROWS), :].astype(f32)
            t0, t1, t2, t3 = (w[r:r + 8] * jnp.tile(act_cols[i][r:r + 8], (1, D // 128))
                              for r in range(0, W2_ROWS, 8))
            out = out + ((t0 + t1) + (t2 + t3))
    o_ref[0] = jnp.sum(out, axis=0, keepdims=True).astype(o_ref.dtype)


@jax.jit
def pallas_sequential_preLN__sliding_block_cached__mixer_channel_mlp__decode_kernel(
    A_x: jax.Array,
    A_k_cache: jax.Array,
    A_v_cache: jax.Array,
    A_wq: jax.Array,
    A_wo: jax.Array,
    B_x: jax.Array,
    B_w1: jax.Array,
    B_b1: jax.Array,
    B_w2: jax.Array,
    B_b2: jax.Array,
):
    del B_x
    cache_len = A_k_cache.shape[2]
    assert A_x.shape == (1, 1, D) and A_wq.shape == (D, HQ * DH) and B_w1.shape == (D, F)
    assert A_k_cache.shape == A_v_cache.shape == (1, HKV, cache_len, DH)
    assert min(4096, max(256, cache_len // 4)) == WINDOW and cache_len % KEYS == 0

    return pl.pallas_call(
        _block_kernel,
        in_specs=[pl.BlockSpec(memory_space=pltpu.HBM)] * 9,
        out_specs=pl.BlockSpec(memory_space=pltpu.VMEM),
        out_shape=jax.ShapeDtypeStruct(A_x.shape, A_x.dtype),
        scratch_shapes=[
            pltpu.VMEM(A_x.shape, A_x.dtype),
            pltpu.VMEM(B_b1.shape, B_b1.dtype),
            pltpu.VMEM(B_b2.shape, B_b2.dtype),
            pltpu.VMEM((N_KV, HKV, KEYS, DH), A_k_cache.dtype),
            pltpu.VMEM((N_KV, HKV, KEYS, DH), A_v_cache.dtype),
            pltpu.VMEM(A_wq.shape, A_wq.dtype),
            pltpu.VMEM((WO_PARTS, HKV, REP * DH // WO_PARTS, D), A_wo.dtype),
            pltpu.VMEM(B_w1.shape, B_w1.dtype),
            pltpu.VMEM(B_w2.shape, B_w2.dtype),
            pltpu.VMEM((HKV, ROWS, DH), jnp.float32),
            pltpu.SemaphoreType.DMA((N_SEMS,)),
        ],
        compiler_params=pltpu.CompilerParams(
            vmem_limit_bytes=48 * 1024 * 1024,
            disable_semaphore_checks=True,
        ),
    )(A_x, A_k_cache, A_v_cache, A_wq, A_wo, B_w1, B_b1, B_w2, B_b2)
```
